```python
import os as _os
_os.environ.setdefault("JAX_PLATFORMS", "cpu")
import jax
import jax.numpy as jnp

def _softmax(x, axis=-1):
    return jax.nn.softmax(x, axis=axis)
def _gelu(x):
    return jax.nn.gelu(x, approximate=True)
def _silu(x):
    return jax.nn.silu(x)
def _sigmoid(x):
    return jax.nn.sigmoid(x)
def _layernorm(x, axis=-1, eps=1e-5):
    m = jnp.mean(x, axis=axis, keepdims=True)
    v = jnp.var(x, axis=axis, keepdims=True)
    return (x - m) / jnp.sqrt(v + eps)
def _scatter_add(tgt, idx, src, axis=0):
    return tgt.at[idx].add(src)
def _segment_sum(src, seg, n):
    return jax.ops.segment_sum(src, seg, n)
class _Rng:
    def __init__(self, key):
        self._k = key
    def _next(self):
        self._k, sub = jax.random.split(self._k)
        return sub
    def normal(self, shape):
        return jax.random.normal(self._next(), shape, dtype=jnp.bfloat16)
    def randint(self, lo, hi, shape):
        return jax.random.randint(self._next(), shape, lo, hi, dtype=jnp.int32)
    def uniform(self, shape, lo=0.0, hi=1.0):
        return jax.random.uniform(self._next(), shape, jnp.bfloat16, lo, hi)
    def permutation(self, n):
        return jax.random.permutation(self._next(), n)


kernel_name = 'gated_mix__linear_attn_block__swiglu_ffn__prompt'

def setup_inputs():
    _rng = _Rng(jax.random.key(int.from_bytes(__import__("os").urandom(4), "little")))
    _w = (lambda a: (lambda t: t.astype(jnp.bfloat16) if jnp.issubdtype(t.dtype, jnp.floating) else t)(jnp.asarray(a)))
    def _A_setup():
        B, S, D = 1, 2048, 512
        return {
            "x": _w((lambda *s: _rng.normal(s) * 0.05)(B, S, D)),
            "wqkv": _w((lambda *s: _rng.normal(s) * 0.8)(D, 3 * D)),
            "wo": _w((lambda *s: _rng.normal(s) * 0.05)(D, D)),
        }
    _A_in = _A_setup()

    def _B_setup():
        B, S, D, F = 1, 2048, 512, 1792
        return {
            "x": _w((lambda *s: _rng.normal(s) * 0.05)(B, S, D)),
            "w_gate": _w((lambda *s: _rng.normal(s) * 0.1)(D, F)),
            "w_up": _w((lambda *s: _rng.normal(s) * 0.1)(D, F)),
            "w_down": _w((lambda *s: _rng.normal(s) * 0.1)(F, D)),
        }
    _B_in = _B_setup()

    return {
        "A_x": _A_in["x"],
        "A_wqkv": _A_in["wqkv"],
        "A_wo": _A_in["wo"],
        "B_x": _B_in["x"],
        "B_w_gate": _B_in["w_gate"],
        "B_w_up": _B_in["w_up"],
        "B_w_down": _B_in["w_down"],
        "gate_w": _w((lambda *s: _rng.normal(s) * 0.05)(512) * 16.0),
    }

def reference(A_x, A_wqkv, A_wo, B_x, B_w_gate, B_w_up, B_w_down, gate_w):
    def _A_ref(x, wqkv, wo):
        B, S, D = x.shape
        H = 32; Dh = D // H
        qkv = (lambda x, *d: x.transpose(*d))((x @ wqkv).reshape(B, S, 3, H, Dh), 2, 0, 3, 1, 4)
        q, k, v = qkv[0], qkv[1], qkv[2]
        phi = lambda t: jnp.where(t > 0, t + 1, jnp.exp(t)) + 1e-6
        pq, pk = phi(q), phi(k)
        kv = jnp.einsum("bhsd,bhse->bhde", pk, v)
        z = jnp.einsum("bhsd->bhd", pk)
        num = jnp.einsum("bhqd,bhde->bhqe", pq, kv)
        den = jnp.einsum("bhqd,bhd->bhq", pq, z)[..., None] + 1e-6
        o = num / den
        return (lambda x, *d: x.transpose(*d))(o, 0, 2, 1, 3).reshape(B, S, D) @ wo

    def _B_ref(x, w_gate, w_up, w_down):
        g = _silu(x @ w_gate)
        u = x @ w_up
        return (g * u) @ w_down

    x = A_x
    g = _sigmoid((x * gate_w).sum(-1, keepdims=True))
    a = _A_ref(x, A_wqkv, A_wo)
    b = _B_ref(x, B_w_gate, B_w_up, B_w_down)
    return g * a + (1 - g) * b
```

```python
import jax
import jax.numpy as jnp
from jax import lax
import jax.experimental.pallas as pl
import jax.experimental.pallas.tpu as pltpu

S, D, F, H = 2048, 512, 1792, 32
DH = D // H
T = 128
R = S // 4
NMXU = 4
NTMP, NBUF = 160, 20
BF, F32, U32 = jnp.bfloat16, jnp.float32, jnp.uint32

CA = ({0: 1, 3: 1}, {2: 1, 3: 1}, {0: 1}, {3: 1}, {0: 1, 1: 1}, {2: 1, 0: -1}, {1: 1, 3: -1})
CB = ({0: 1, 3: 1}, {0: 1}, {1: 1, 3: -1}, {2: 1, 0: -1}, {3: 1}, {0: 1, 1: 1}, {2: 1, 3: 1})
CC = ({0: 1, 3: 1}, {2: 1, 3: -1}, {1: 1, 3: 1}, {0: 1, 2: 1}, {1: 1, 0: -1}, {3: 1}, {0: 1})
LAM = (0.0, 1.0, -1.0, 2.0)

WQT, WQ, Z, PKX, KV, W2, NSQ = 0, 4, 8, 9, 13, 14, 18
PRE_K, PRE_Q, HID_Q = 12, 16, 14


def _comb(coef, get):
    out = None
    for k, s in coef.items():
        v = get(k)
        out = v if out is None else (out + v if s > 0 else out - v)
    return out


def _rc(k1, k2):
    return 2 * (k1 // 2) + k2 // 2, 2 * (k1 % 2) + k2 % 2


def _comb2(table, i, j, blk):
    return _comb(table[j], lambda k2: _comb(table[i], lambda k1: blk(*_rc(k1, k2))))


class _Quad(list):
    def __add__(self, other):
        return _Quad(a + b for a, b in zip(self, other))

    def __sub__(self, other):
        return _Quad(a - b for a, b in zip(self, other))


def _strassen_rounds(prods, left, keep):
    if left == 3:
        m2, m4, m1 = prods(1, 3, 0)
        c21, t1, t2 = m2 + m4, keep(m1 + m4), keep(m1 - m2)
        m3, m5, m7, m6 = prods(2, 4, 6, 5)
        return _Quad([(m7 - m5) + t1(), m3 + m5, c21, (m3 + m6) + t2()])
    if left == 1:
        m7 = keep(prods(6)[0])
    if left == 2:
        m1, m7 = prods(0, 6)
        y, m1 = keep(m1 + m7), keep(m1)
    m2, m4, m3, m5 = prods(1, 3, 2, 4)
    c21, c12, t1, t2 = m2 + m4, m3 + m5, m4 - m5, m3 - m2
    if left == 2:
        c11, t2 = t1 + y(), keep(t2 + m1())
        return _Quad([c11, c12, c21, prods(5)[0] + t2()])
    if left == 1:
        t1, t2 = keep(t1 + m7()), keep(t2)
        m1, m6 = prods(0, 5)
        return _Quad([m1 + t1(), c12, c21, (m1 + m6) + t2()])
    t1, t2 = keep(t1), keep(t2)
    m1, m7, m6 = prods(0, 6, 5)
    return _Quad([(m1 + m7) + t1(), c12, c21, (m1 + m6) + t2()])


def _strassen_steps(prod, emit, keep):
    m3 = keep(prod(2))
    yield
    m5 = prod(4)
    emit(1, m5 + m3())
    m5 = keep(m5)
    yield
    m4 = keep(prod(3))
    yield
    m2 = prod(1)
    emit(2, m2 + m4())
    t2 = keep(m3() - m2)
    yield
    m1 = keep(prod(0))
    yield
    emit(0, ((prod(6) + m1()) + m4()) - m5())
    yield
    emit(3, (prod(5) + m1()) + t2())
    yield


def _strassen_dual(prod, keep):
    m1 = keep(prod(0))
    b11 = keep(prod(1) + m1())
    m4 = prod(3)
    b11, m4 = keep(b11() - m4), keep(m4)
    m7 = prod(6)
    b21, b22 = m7 + m4(), keep(m7 + m1())
    b22 = keep(prod(4) + b22())
    m3 = prod(2)
    b22, m3 = b22() - m3, keep(m3)
    m6 = prod(5)
    return [m6 + b11(), m6 + m3(), b21, b22]


def _hopcroft_kerr(a, b, keep):
    def axpy(s, x, y):
        return y if s == 0 else y + x if s == 1 else y - x if s == -1 else y + s * x

    def mm(x, y):
        return _dot(x.astype(BF), y.astype(BF))

    def cross(i, j):
        x = axpy(-LAM[j], a(i, 0), axpy(LAM[j], a(j, 0), a(j, 1)) - a(i, 1))
        y = axpy(-LAM[i], b(1, j) - b(1, i), b(0, j) - b(0, i)) * (1 / (LAM[i] - LAM[j]))
        return mm(x, y)

    p, q, c = {}, {}, {}
    for i in range(4):
        pi = mm(a(i, 0), axpy(-LAM[i], b(1, i), b(0, i)))
        qi = mm(axpy(LAM[i], a(i, 0), a(i, 1)), b(1, i))
        p[i], q[i], c[i, i] = keep(pi), keep(qi), keep(pi + qi)
    pairs = [(i, j) for i in range(4) for j in range(i)]
    ops = [(axpy(-LAM[j], a(j, 0), axpy(LAM[i], a(i, 0), a(i, 1)) - a(j, 1)),
            (axpy(-LAM[i], b(1, i), b(0, i)) - axpy(-LAM[j], b(1, j), b(0, j))) * (1 / (LAM[i] - LAM[j])))
           for i, j in pairs]
    halves = [[mm(x[s:s + R // 2], y) for x, y in ops[:2]] for s in (0, R // 2)]
    early = [keep(jnp.concatenate(v, axis=0)) for v in zip(*halves)]
    for n, ((i, j), (x, y)) in enumerate(zip(pairs[2:], ops[2:])):
        m = mm(x, y)
        c[i, j] = keep(((cross(i, j) - m) + p[i]()) + q[j]())
        c[j, i] = keep(((cross(j, i) + m) + p[j]()) + q[i]())
        i, j = pairs[n // 2]
        if n % 2:
            c[i, j] = keep(((cross(i, j) - early[n // 2]()) + p[i]()) + q[j]())
        else:
            c[j, i] = keep(((cross(j, i) + early[n // 2]()) + p[j]()) + q[i]())
    return c


def _elu1(t):
    return jnp.where(t > 0, t + 1.0, jnp.exp(t))


def _silu_of_twice(half):
    return half * jnp.tanh(half) + half


def _dot(a, b):
    return jnp.dot(a, b, preferred_element_type=F32)


def _rows(r):
    return slice(r * R, (r + 1) * R)


def _tile(c):
    return slice(c * T, (c + 1) * T)


def _rep(v, n):
    return jnp.concatenate([v] * (n // 8), axis=0)


def _run(steps):
    for _ in steps:
        pass


def _kernel(x_hbm, wqkv_hbm, wo_hbm, wg_hbm, wu_hbm, wd_hbm, gw_hbm, o_hbm,
            x_v, wqkv_v, wo_v, wg_v, wu_v, wd_v, gw_v,
            xa_v, pkt_v, sq_v, gate_v, h_v, pre_v, o_v, sems, *tmp_v):
    def x_quad(k):
        return x_hbm, x_v, (slice(k // 2 * S // 2, (k // 2 + 1) * S // 2), slice(k % 2 * D // 2, (k % 2 + 1) * D // 2))

    def wqkv_cols(c, n=2):
        return wqkv_hbm, wqkv_v, (slice(None), slice(c * T, (c + n) * T))

    def wu_cols(c):
        return wu_hbm, wu_v, (slice(None), slice(c * T, (c + 2) * T))

    everything = (slice(None), slice(None))
    stages = [
        [x_quad(0), wqkv_cols(6)],
        [wu_cols(2)],
        [x_quad(1)],
        [wu_cols(6), wu_cols(10)],
        [x_quad(3), wqkv_cols(4), wu_cols(0), wu_cols(4), x_quad(2)],
        [wu_cols(8), wqkv_cols(0, 4), (wg_hbm, wg_v, everything), wqkv_cols(8, 4), (wo_hbm, wo_v, everything),
         wu_cols(12), (wd_hbm, wd_v, everything), (gw_hbm, gw_v, everything[:1])],
    ]
    stages = [[pltpu.make_async_copy(src.at[idx], dst.at[idx], sems.at[n]) for src, dst, idx in stage]
              for n, stage in enumerate(stages)]
    for stage in stages:
        for copy in stage:
            copy.start()

    def touch(i, acc):
        for ref in (xa_v, pkt_v, sq_v, gate_v, h_v, pre_v) + tmp_v:
            ref[ref.shape[0] - 1 - i, 0:8, 0:T] = jnp.zeros((8, T), ref.dtype)
        return acc + i
    zero = lax.fori_loop(0, 2, touch, -1)

    state = dict(issued=0, kept=0, last=None, fence=False)
    queues, released, prepared = [], [], []

    def keep(v):
        if isinstance(v, list):
            parts = [keep(a) for a in v]
            return lambda: _Quad(a() for a in parts)
        t, n = state['kept'], v.shape[0]
        state['kept'] += 1
        buf, k = divmod(t % NTMP, NTMP // NBUF)
        buf = tmp_v[buf]
        buf[k, 0:n, :] = v

        def reload():
            assert state['kept'] - t <= NTMP
            state['last'] = buf, k
            if state['fence']:
                state['fence'] = False
                return jnp.concatenate([buf[k, 0:8, :] + gate_v[2 + zero, 0:8, :], buf[k, 8:n, :]], axis=0)
            return buf[k, 0:n, :]
        return reload

    def spread(tasks, steps):
        queues.append([tasks[len(tasks) * s // steps:len(tasks) * (s + 1) // steps] for s in range(steps)])

    def side_work():
        released.append(state['last'])
        if len(released) < 2:
            return
        buf, k = released.pop(0)
        todo = [((n + 0.5) / len(ts), t) for ts in [q.pop(0) for q in queues if q] for n, t in enumerate(ts)]
        for n, (_, task) in enumerate(sorted(todo, key=lambda a: a[0])):
            def late(v, s=n * (R // 8) // len(todo) * 8):
                buf[k, s:s + 8, :] = jnp.full((8, T), v, F32)
                return buf[k, s:s + 8, :]
            task(late)

    def align(steps):
        state['issued'] = -(7 * steps % NMXU)

    def wait(steps):
        assert state['issued'] % NMXU == 0
        align(steps)
        for copy in stages.pop(0):
            copy.wait()

    def xa(i, j, lo=0, hi=R):
        if i not in prepared:
            prepared.append(i)
            block = lambda r, c: x_v[_rows(r), _tile(c)].astype(F32)
            outer = [keep(_comb(CA[i], lambda k1: block(*_rc(k1, k2))))() for k2 in range(4)]
            for n in range(7):
                xa_v[7 * i + n] = pltpu.bitcast(_comb(CA[n], lambda k2: outer[k2]).astype(BF), U32)
        return pltpu.bitcast(xa_v[7 * i + j, lo // 2:hi // 2, :], BF)

    def x_times(wblk, emit, scale=None):
        def weight(i, j):
            if scale is None and len(CB[i]) == 1 and len(CB[j]) == 1:
                return _comb2(CB, i, j, wblk).astype(BF)
            w = _comb2(CB, i, j, lambda r, c: wblk(r, c).astype(F32))
            return (w if scale is None else w * scale).astype(BF)

        def prods(i, js):
            short = state['issued'] < 0
            state['issued'] += len(js)
            ws = [weight(i, j) for j in js]
            cuts = {1: (0, 1, 2, 3, 4), 2: (0, 2, 4), 3: (0, 3, 4)}[len(js)] if short else (0, 4)
            ps = [[_dot(xa(i, j, lo * R // 4, hi * R // 4), w) for j, w in zip(js, ws)] for lo, hi in zip(cuts, cuts[1:])]
            return [jnp.concatenate(p, axis=0) if short else p[0] for p in zip(*ps)]

        def prod(i):
            state['fence'] = not stages
            p = _strassen_rounds(lambda *js: prods(i, js), NMXU - state['issued'] % NMXU, keep)
            side_work()
            return p
        return _strassen_steps(prod, emit, keep)

    def project(wblk, c0, f):
        def emit(k1, val):
            for k2 in range(4):
                r, c = _rc(k1, k2)
                pre_v[c0 + c, _rows(r), :] = f(val[k2])
        return x_times(wblk, emit)

    def up(c0):
        return project(lambda r, c: wu_v[_tile(r), _tile(c0 + c)], c0, lambda v: v)

    def hidden(c0):
        def emit(k1, val):
            for k2 in range(4):
                r, c = _rc(k1, k2)
                u = pre_v[c0 + c, _rows(r), :]
                h_v[c0 + c, _rows(r), :] = (_silu_of_twice(val[k2]) * gate_v[1, _rows(r), :]) * u
        return x_times(lambda r, c: wg_v[_tile(r), _tile(c0 + c)], emit, 0.5)

    def hidden_rest():
        def emit(k1, val):
            for r2 in range(2):
                r = 2 * (k1 // 2) + r2
                h = _silu_of_twice(0.5 * val[2 * r2]) * (val[2 * r2 + 1] * gate_v[1, _rows(r), :])
                h_v[12 + k1 % 2, _rows(r), :] = h
        return x_times(lambda r, c: (wu_v if c % 2 else wg_v)[_tile(r), _tile(12 + c // 2)], emit)

    def by_feature(slot, t):
        return jnp.concatenate([sq_v[slot, pl.ds(4 * t + d, H, stride=DH), :] for d in range(4)], axis=0)

    k = project(lambda r, c: wqkv_v[_tile(r), _tile(4 + c)], PRE_K, _elu1)
    u0, u1, u2 = up(0), up(4), up(8)
    for steps in ([k], [u0], [u0, k], [u1, u1, u2, u2], [u0, k, u1] * 5, []):
        wait(len(steps))
        for g in steps:
            next(g)

    half_gw = 0.5 * gw_v[...].astype(F32).reshape(1, D)

    def gate_task(s, n, late):
        one = late(1.0)
        y = [x_v[s:s + n, _tile(c)].astype(F32) * _rep(one * half_gw[:, _tile(c)], n) for c in range(4)]
        y = jnp.sum((y[0] + y[1]) + (y[2] + y[3]), axis=-1, keepdims=True)
        t = 0.5 * jnp.tanh(jnp.broadcast_to(y, (n, T)))
        gate_v[0, s:s + n, :] = 0.5 + t
        gate_v[1, s:s + n, :] = 0.5 - t

    def wq_task(r, late):
        one = _rep(late(1.0), T)
        for c in range(4):
            sq_v[WQT + r, _tile(c), :] = (wqkv_v[_tile(r), _tile(c)].astype(F32) * one).T
        for t in range(4):
            sq_v[WQ + r, _tile(t), :] = by_feature(WQT + r, t).T

    spread([lambda late, s=s: gate_task(s, 64, late) for s in range(0, S, 64)], 7)
    spread([lambda late, r=r: wq_task(r, late) for r in range(4)], 4)
    _run(u2)

    def pk_task(r, c, n, late):
        pk = pre_v[PRE_K + c, r * R + n * T:r * R + (n + 1) * T, :] + _rep(late(1e-6), T)
        pkt_v[4 * r + c, :, _tile(n)] = pk.T

    spread([lambda late, r=r, c=c, n=n: pk_task(r, c, n, late)
            for r in range(4) for c in range(4) for n in range(4)], 7)
    _run(project(lambda r, c: sq_v[WQ + r, _tile(c), :], PRE_Q, lambda v: _elu1(v) + 1e-6))
    assert not any(queues)

    for c in range(4):
        sq_v[Z, _tile(c), :] = _comb({n: 1 for n in range(16)}, lambda n: pkt_v[4 * (n // 4) + c, :, _tile(n % 4)])
    z = [jnp.sum(by_feature(Z, t).T, axis=0, keepdims=True) for t in range(4)]

    def pkx_prod(i):
        lhs = lambda j: _comb2(CC, i, j, lambda r, c: pkt_v[4 * r + c]).astype(BF)
        return jnp.concatenate(_strassen_dual(lambda j: _dot(lhs(j), xa(i, j)), keep), axis=0)

    for k1, v in enumerate(_strassen_dual(pkx_prod, keep)):
        sq_v[PKX + k1, 0:D, :] = v
    align(0)

    def norm_task(s, n, late):
        pq = [pre_v[PRE_Q + c, s:s + n, :] for c in range(4)]
        one = late(1.0)
        y = [pq[c] * _rep(one * z[c], n) for c in range(4)]
        y = (y[0] + y[1]) + (y[2] + y[3])
        y = y + pltpu.roll(y, 2 * H, 1)
        y = y + pltpu.roll(y, H, 1)
        scale = gate_v[0, s:s + n, :] / (y + 1e-6)
        for c in range(4):
            h_v[HID_Q + c, s:s + n, :] = pq[c] * scale

    spread([lambda late, s=s: norm_task(s, 32, late) for s in range(0, S, 32)], 13)
    _run(hidden(0))

    head = lambda axis: lax.broadcasted_iota(jnp.int32, (T, T), axis) // DH
    same_head = head(0) == head(1)
    for c in range(4):
        m = jnp.concatenate([sq_v[PKX + 2 * (r // 2) + c // 2, _tile(2 * (r % 2) + c % 2), :] for r in range(4)], axis=1)
        sq_v[KV, _tile(c), :] = jnp.where(same_head, _dot(m.astype(BF), wqkv_v[:, _tile(8 + c)]), 0.0)
    align(0)
    _run(hidden(4))
    _run(hidden(8))

    for c in range(4):
        kv = jnp.concatenate([sq_v[KV, pl.ds(c * T + d, 8, stride=DH), :] for d in range(DH)], axis=0).astype(BF)
        for n in range(4):
            w = _dot(kv, wo_v[_tile(c), _tile(n)])
            for d in range(DH):
                sq_v[W2 + n, d * H + 8 * c:d * H + 8 * c + 8, :] = w[8 * d:8 * d + 8]
    align(7)
    _run(hidden_rest())
    assert not any(queues)

    out_copies = []

    def write(k1, val):
        for k2 in (1, 2, 0, 3):
            r, c = _rc(k1, k2)
            n = R // 4 if (r, c) == (3, 3) else R
            for s in range(0, R, n):
                o_v[4 * r + c, s:s + n, :] = val[k2][s:s + n].astype(BF)
                copy = pltpu.make_async_copy(o_v.at[4 * r + c, s:s + n, :],
                                             o_hbm.at[r * R + s:r * R + s + n, _tile(c)], sems.at[0])
                copy.start()
                out_copies.append(copy)

    def out_prod(i):
        def prod(j):
            a = [_comb2(CA, i, j, lambda r, c: h_v[b + c, _rows(r), :]) for b in (HID_Q, 0, 4, 8)]
            w = [_comb2(CB, i, j, lambda r, c: sq_v[W2 + c, _tile(r), :])]
            w += [_comb2(CB, i, j, lambda r, c: wd_v[_tile(b + r), _tile(c)].astype(F32)) for b in (0, 4, 8)]
            return _dot(jnp.concatenate(a, axis=1).astype(BF), jnp.concatenate(w, axis=0).astype(BF))
        done = {}
        _run(_strassen_steps(prod, done.setdefault, keep))
        return _Quad(done[k2] for k2 in range(4))

    m3 = keep(out_prod(2))
    rest = _hopcroft_kerr(lambda i, n: h_v[12 + n, _rows(i), :],
                          lambda n, j: wd_v[_tile(12 + n), _tile(j)].astype(F32), keep)
    rest_quad = lambda k1: _Quad(rest[_rc(k1, k2)]() for k2 in range(4))
    m5 = out_prod(4)
    write(1, (m5 + m3()) + rest_quad(1))
    t1 = keep(rest_quad(0) - m5)
    m4 = keep(out_prod(3))
    m2 = out_prod(1)
    write(2, (m2 + m4()) + rest_quad(2))
    t2 = keep((m3() - m2) + rest_quad(3))
    m1 = out_prod(0)
    t1, t2 = keep((m1 + t1()) + m4()), keep(m1 + t2())
    write(0, out_prod(6) + t1())
    write(3, out_prod(5) + t2())
    for copy in out_copies:
        copy.wait()


@jax.jit
def pallas_gated_mix__linear_attn_block__swiglu_ffn__prompt_kernel(
    A_x: jax.Array,
    A_wqkv: jax.Array,
    A_wo: jax.Array,
    B_x: jax.Array,
    B_w_gate: jax.Array,
    B_w_up: jax.Array,
    B_w_down: jax.Array,
    gate_w: jax.Array,
):
    del B_x
    in_hbm = pl.BlockSpec(memory_space=pl.ANY)
    out = pl.pallas_call(
        _kernel,
        out_shape=jax.ShapeDtypeStruct((S, D), BF),
        in_specs=[in_hbm] * 7,
        out_specs=in_hbm,
        scratch_shapes=[
            pltpu.VMEM((S, D), BF), pltpu.VMEM((D, 3 * D), BF), pltpu.VMEM((D, D), BF),
            pltpu.VMEM((D, F), BF), pltpu.VMEM((D, F), BF), pltpu.VMEM((F, D), BF), pltpu.VMEM((D,), BF),
            pltpu.VMEM((49, R // 2, T), U32),
            pltpu.VMEM((16, T, R), F32),
            pltpu.VMEM((NSQ, D + DH, T), F32),
            pltpu.VMEM((3, S, T), F32),
            pltpu.VMEM((18, S, T), F32),
            pltpu.VMEM((20, S, T), F32),
            pltpu.VMEM((16, R, T), BF),
            pltpu.SemaphoreType.DMA((6,)),
        ] + [pltpu.VMEM((NTMP // NBUF, R, T), F32)] * NBUF,
        compiler_params=pltpu.CompilerParams(
            vmem_limit_bytes=120 * 1024 * 1024, disable_semaphore_checks=True, disable_bounds_checks=True),
    )(A_x.reshape(S, D), A_wqkv, A_wo, B_w_gate, B_w_up, B_w_down, gate_w)
    return out.reshape(1, S, D)
```
